```python
import os as _os
_os.environ.setdefault('JAX_PLATFORMS', 'cpu')
import jax
import jax.numpy as jnp

def _softmax(x, axis=-1):
    return jax.nn.softmax(x, axis=axis)

def _gelu(x):
    return jax.nn.gelu(x, approximate=True)

def _silu(x):
    return jax.nn.silu(x)

def _sigmoid(x):
    return jax.nn.sigmoid(x)

def _layernorm(x, axis=-1, eps=1e-05):
    m = jnp.mean(x, axis=axis, keepdims=True)
    v = jnp.var(x, axis=axis, keepdims=True)
    return (x - m) / jnp.sqrt(v + eps)

def _scatter_add(tgt, idx, src, axis=0):
    return tgt.at[idx].add(src)

def _segment_sum(src, seg, n):
    return jax.ops.segment_sum(src, seg, n)

class _Rng:

    def __init__(self, key):
        self._k = key

    def _next(self):
        self._k, sub = jax.random.split(self._k)
        return sub

    def normal(self, shape):
        return jax.random.normal(self._next(), shape, dtype=jnp.bfloat16)

    def randint(self, lo, hi, shape):
        return jax.random.randint(self._next(), shape, lo, hi, dtype=jnp.int32)

    def uniform(self, shape, lo=0.0, hi=1.0):
        return jax.random.uniform(self._next(), shape, jnp.bfloat16, lo, hi)

    def permutation(self, n):
        return jax.random.permutation(self._next(), n)
kernel_name = 'adaLN_cond__linear_attn_block__swiglu_ffn__prompt'

def setup_inputs():
    _rng = _Rng(jax.random.key(int.from_bytes(__import__("os").urandom(4), "little")))
    _w = lambda a: (lambda t: t.astype(jnp.bfloat16) if jnp.issubdtype(t.dtype, jnp.floating) else t)(jnp.asarray(a))

    def _A_setup():
        B, S, D = (1, 2048, 640)
        return {'x': _w((lambda *s: _rng.normal(s) * 0.05)(B, S, D)), 'wqkv': _w((lambda *s: _rng.normal(s) * 0.8)(D, 3 * D)), 'wo': _w((lambda *s: _rng.normal(s) * 0.05)(D, D))}
    _A_in = _A_setup()

    def _B_setup():
        B, S, D, F = (1, 2048, 640, 1728)
        return {'x': _w((lambda *s: _rng.normal(s) * 0.05)(B, S, D)), 'w_gate': _w((lambda *s: _rng.normal(s) * 0.05)(D, F)), 'w_up': _w((lambda *s: _rng.normal(s) * 0.05)(D, F)), 'w_down': _w((lambda *s: _rng.normal(s) * 0.05)(F, D))}
    _B_in = _B_setup()
    return {'A_x': _A_in['x'], 'A_wqkv': _A_in['wqkv'], 'A_wo': _A_in['wo'], 'B_x': _B_in['x'], 'B_w_gate': _B_in['w_gate'], 'B_w_up': _B_in['w_up'], 'B_w_down': _B_in['w_down'], 'c': _w((lambda *s: _rng.normal(s) * 0.05)(1, 640) * 8.0), 'w_mod': _w((lambda *s: _rng.normal(s) * 0.05)(640, 6 * 640) * 640 ** (-0.5) * 8.0)}

def reference(A_x, A_wqkv, A_wo, B_x, B_w_gate, B_w_up, B_w_down, c, w_mod):

    def _A_ref(x, wqkv, wo):
        B, S, D = x.shape
        H = 32
        Dh = D // H
        qkv = (lambda x, *d: x.transpose(*d))((x @ wqkv).reshape(B, S, 3, H, Dh), 2, 0, 3, 1, 4)
        q, k, v = (qkv[0], qkv[1], qkv[2])
        phi = lambda t: jnp.where(t > 0, t + 1, jnp.exp(t)) + 1e-06
        pq, pk = (phi(q), phi(k))
        kv = jnp.einsum('bhsd,bhse->bhde', pk, v)
        z = jnp.einsum('bhsd->bhd', pk)
        num = jnp.einsum('bhqd,bhde->bhqe', pq, kv)
        den = jnp.einsum('bhqd,bhd->bhq', pq, z)[..., None] + 1e-06
        o = num / den
        return (lambda x, *d: x.transpose(*d))(o, 0, 2, 1, 3).reshape(B, S, D) @ wo

    def _B_ref(x, w_gate, w_up, w_down):
        g = _silu(x @ w_gate)
        u = x @ w_up
        return g * u @ w_down
    x = A_x
    mod = (_silu(c) @ w_mod).reshape(c.shape[0], 6, 1, -1)
    sa, ca, ga, sb, cb, gb = (mod[:, 0].copy(), mod[:, 1].copy(), mod[:, 2].copy(), mod[:, 3].copy(), mod[:, 4].copy(), mod[:, 5].copy())
    h = _layernorm(x, axis=-1) * (1 + ca) + sa
    x = x + ga * _A_ref(h, A_wqkv, A_wo)
    h = _layernorm(x, axis=-1) * (1 + cb) + sb
    x = x + gb * _B_ref(h, B_w_gate, B_w_up, B_w_down)
    return x
```

```python
import functools
import itertools

import jax
import jax.numpy as jnp
import numpy as np
from jax import lax
import jax.experimental.pallas as pl
import jax.experimental.pallas.tpu as pltpu

F32, BF16, U32 = jnp.float32, jnp.bfloat16, jnp.uint32
T = 128
NT = 5
HEADS = 32
R1, R2 = 256, 128

_SCHEME = """
0+00000000 +-00000000 -000+00000-0000-000000000
++00000000 +000000000 +0--0000000000000000+0000
000+000000 00+-000000 0-000--00+0-0000-00000000
00++000000 00+0000000 0+000-+--000000000000+000
0000++0000 00000+0000 0000000000--+000000000+00
0000+00000 0000+-0000 00+0000+0000+0-0000000000
000000++00 0000000+00 0000000000000+0---+0000+0
000000+000 000000+-00 000+0000+0000+000++-00000
00000000+0 00000000+0 0000+-000+000-00000000--+
000000000+ 000000000+ 0-000000000000+00-0+--00+
+000-00000 +000+00000 00+0000000000000000000000
0+000-0000 0+000+0000 0000000000-00000000000000
0+00+00000 +0000+0000 00+0000000+00000000000000
+00000-000 +00000+000 000+000000000000000000000
0+00000-00 0+00000+00 000000000000000-000000000
0+0000+000 +000000+00 000+00000000000+000000000
++000000-- 0+0000000+ 0-000000000000000000-0000
+0000000-0 +-000000+- 0000++0000000000000000000
++000000-0 +-0000000- 0000-000000000000000-0000
00+0-00000 00+0+00000 0000000+00000000000000000
000+0-0000 000+0+0000 00000000000-0000000000000
000++00000 00+00+0000 0000000+000+0000000000000
00+000-000 00+000+000 00000000+0000000000000000
000+000-00 000+000+00 0000000000000000-00000000
000+00+000 00+0000+00 00000000+0000000+00000000
00++0000-- 000+00000+ 0-0000000000000000000-000
00+00000-0 00+-0000+- 00000-000+000000000000000
00++0000-0 00+-00000- 0-000+000-00000000000-000
00000+000- 0000+-00+- 00000000000000-00-0000000
0000++00-- 0000+000+0 0000000000000-00000000-00
0000++000- 0000+-00+0 00000000000000+0000000+00
0000000+0- 000000+-+- 00000000000000000+0-00000
000000++-- 000000+0+0 0000000000000-000000000-0
000000++0- 000000+-+0 0000000000000+000-0+000+0
+0-00000-0 +0+00000+0 00000-0000000000000000000
0+0-00000- 0+0+00000+ 0+00000000000000000000000
+00+0000-0 0++000000+ 0+000+0000000000000000000
0000+0-0-0 0000+0+0+0 0000000000000+00000000000
00000+0-0- 00000+0+0+ 00000000000000000-0000000
00000++00- 0000+00++0 0000000000000+000+0000000
"""


def _parse(table):
    rows = [line.split() for line in table.strip().splitlines()]
    u, x, c = (np.array([["-0+".index(ch) - 1 for ch in row[i]] for row in rows]) for i in range(3))
    for p in range(len(rows)):
        if not (c[p] > 0).any():
            c[p], x[p] = -c[p], -x[p]
    return u, x, c


_U, _X, _C = _parse(_SCHEME)
P = len(_U)


def _by_columns(cols):
    used = [np.nonzero(np.abs(_X[p]).reshape(NT, 2).sum(1))[0] for p in range(P)]
    return sorted(range(P), key=lambda p: (sorted(cols.index(c) for c in used[p]), p))


_ORDER = {
    'G': (8, 9, 28, 29, 30, 37, 38, 39, 16, 17, 18, 35, 36, 31, 32, 33, 25, 34, 26, 27,
          4, 5, 10, 11, 12, 19, 20, 21, 0, 1, 13, 14, 15, 6, 7, 22, 23, 24, 2, 3),
    'a': (18, 8, 17, 35, 16, 9, 36, 25, 26, 27, 30, 37, 34, 28, 29, 38, 39, 1, 0, 31,
          13, 14, 33, 10, 11, 12, 21, 19, 32, 20, 15, 2, 22, 23, 3, 24, 4, 5, 6, 7),
    'd': (8, 9, 16, 17, 18, 7, 34, 36, 25, 26, 0, 27, 30, 13, 11, 38, 32, 28, 14, 20,
          12, 39, 37, 21, 23, 15, 22, 19, 5, 29, 10, 31, 2, 33, 4, 6, 24, 35, 3, 1),
    'g': (23, 16, 8, 17, 3, 19, 9, 34, 18, 35, 36, 26, 25, 27, 29, 10, 28, 11, 12, 20,
          30, 32, 14, 39, 1, 33, 13, 37, 31, 38, 21, 2, 22, 6, 15, 7, 0, 24, 4, 5),
    'k': (8, 9, 16, 17, 18, 34, 35, 36, 31, 32, 33, 37, 38, 39, 28, 29, 30, 25, 26, 27,
          0, 1, 13, 14, 15, 10, 11, 12, 6, 7, 22, 23, 24, 4, 5, 19, 20, 21, 2, 3),
    'k0': (8, 9, 31, 32, 36, 33, 37, 38, 39, 16, 17, 18, 34, 35, 28, 29, 30, 25, 26, 27,
          6, 7, 13, 14, 15, 22, 23, 24, 0, 1, 10, 11, 12, 4, 5, 19, 20, 21, 2, 3),
    'k1': (8, 9, 2, 16, 17, 18, 34, 35, 36, 28, 29, 30, 37, 38, 39, 31, 32, 33, 25, 26,
          27, 0, 1, 10, 11, 12, 13, 14, 15, 4, 5, 19, 20, 21, 6, 7, 22, 23, 24, 3),
    'k3': _by_columns((4, 1, 3, 2, 0)),
    'k7': (8, 9, 25, 26, 27, 34, 35, 36, 31, 32, 33, 37, 38, 39, 16, 17, 18, 28, 29, 30,
          2, 3, 22, 23, 24, 19, 20, 21, 6, 7, 13, 14, 15, 0, 1, 10, 11, 12, 4, 5),
    'q': (30, 26, 8, 9, 25, 29, 27, 34, 35, 36, 16, 17, 18, 28, 37, 38, 39, 31, 32, 33,
          2, 3, 19, 20, 21, 22, 23, 24, 0, 1, 10, 11, 12, 13, 14, 15, 4, 5, 6, 7),
    'q0': (2, 3, 22, 23, 24, 25, 26, 27, 34, 35, 36, 19, 31, 33, 20, 21, 6, 38, 39, 13,
          32, 7, 14, 37, 15, 8, 9, 28, 29, 30, 16, 17, 18, 4, 5, 10, 11, 12, 0, 1),
    'q1': (4, 5, 19, 20, 21, 37, 38, 39, 10, 12, 11, 28, 29, 30, 2, 3, 22, 23, 24, 34,
          35, 36, 25, 26, 27, 6, 7, 13, 14, 15, 31, 32, 33, 0, 1, 16, 17, 18, 8, 9),
    'q2': (8, 9, 16, 17, 18, 34, 36, 35, 25, 26, 27, 28, 29, 30, 37, 38, 39, 31, 32, 33,
          0, 1, 10, 11, 13, 12, 14, 15, 2, 3, 19, 20, 21, 22, 23, 24, 4, 5, 6, 7),
    'q3': (2, 3, 22, 23, 19, 20, 21, 34, 35, 36, 25, 26, 27, 6, 7, 37, 38, 24, 39, 13,
          14, 15, 31, 32, 33, 4, 5, 10, 11, 12, 28, 29, 30, 0, 1, 16, 17, 18, 8, 9),
    'q4': (16, 17, 18, 0, 1, 34, 35, 36, 10, 11, 12, 14, 15, 8, 9, 29, 30, 37, 28, 38,
          39, 25, 26, 27, 31, 32, 33, 4, 5, 19, 20, 21, 2, 3, 13, 22, 23, 24, 6, 7),
    'q5': (20, 21, 34, 35, 2, 16, 3, 19, 36, 25, 26, 27, 22, 23, 24, 4, 5, 30, 12, 28,
          10, 11, 29, 37, 17, 9, 31, 32, 38, 39, 0, 1, 6, 7, 18, 13, 14, 15, 8, 33),
    'q6': (4, 5, 28, 29, 30, 37, 38, 39, 10, 11, 12, 9, 16, 19, 20, 21, 8, 17, 18, 34,
          35, 36, 25, 26, 27, 31, 32, 33, 0, 1, 13, 14, 15, 2, 3, 22, 23, 24, 6, 7),
    'q7': (34, 2, 3, 35, 0, 1, 36, 22, 23, 24, 26, 27, 19, 20, 21, 12, 6, 13, 14, 15,
          16, 17, 18, 10, 11, 7, 31, 37, 25, 38, 39, 8, 32, 33, 9, 28, 29, 30, 4, 5),
    'u': (14, 38, 8, 36, 39, 18, 9, 16, 15, 30, 17, 35, 34, 13, 25, 26, 33, 10, 5, 29,
          1, 2, 37, 31, 0, 11, 12, 3, 32, 27, 28, 19, 20, 21, 22, 23, 4, 6, 24, 7),
}


def _signed_sum(terms):
    terms = sorted(((v, s) for v, s in terms if v is not None), key=lambda t: -t[1])
    if not terms:
        return None
    acc = terms[0][0] if terms[0][1] > 0 else -terms[0][0]
    for v, s in terms[1:]:
        acc = acc + v if s > 0 else acc - v
    return acc


class _Sums:
    def __init__(self, signs, share=True):
        self.rows = [{j: int(s) for j, s in enumerate(row) if s} for row in signs]
        self.steps = {}
        new = signs.shape[1]
        while share:
            count = {}
            for row in self.rows:
                for a, b in itertools.combinations(sorted(row), 2):
                    key = (a, b, row[a] * row[b])
                    count[key] = count.get(key, 0) + 1
            top = max(count.values(), default=0)
            if top < 2:
                break
            a, b, s = self.steps[new] = min(key for key, n in count.items() if n == top)
            for row in self.rows:
                if a in row and b in row and row[a] * row[b] == s:
                    row[new] = row.pop(a)
                    del row[b]
            new += 1

    def of(self, inputs):
        vals = dict(enumerate(inputs))

        def val(j):
            if j not in vals:
                a, b, s = self.steps[j]
                vals[j] = _signed_sum([(val(a), 1), (val(b), s)])
            return vals[j]

        for row in self.rows:
            yield _signed_sum([(val(j), s) for j, s in sorted(row.items())])

    def stream(self):
        vals, pending = {}, dict(self.steps)
        left = [dict(row) for row in self.rows]
        acc = [None] * len(left)

        def push(j, value):
            vals[j] = value
            ready = True
            while ready:
                ready = False
                for k, (a, b, s) in sorted(pending.items()):
                    if a in vals and b in vals:
                        vals[k] = vals[a] + vals[b] if s > 0 else vals[a] - vals[b]
                        del pending[k]
                        ready = True
            done = []
            for i, todo in enumerate(left):
                if not todo:
                    continue
                for k in sorted(todo, key=lambda k: -todo[k]):
                    if k in vals:
                        s = todo.pop(k)
                        if acc[i] is None:
                            acc[i] = (vals[k], s)
                        elif acc[i][1] > 0:
                            acc[i] = (acc[i][0] + vals[k] if s > 0 else acc[i][0] - vals[k], 1)
                        else:
                            acc[i] = (vals[k] - acc[i][0], 1) if s > 0 else (acc[i][0] + vals[k], -1)
                if not todo:
                    done.append((i, acc[i][0] if acc[i][1] > 0 else -acc[i][0]))
            return done

        return push


def _once(fn, *args):
    fn(*args)
    yield from ()


def _chain(*steps):
    total, base = sum(w for w, _ in steps), 0.0
    for w, step in steps:
        for f in step:
            yield (base + f * w) / total
        base += w


def _issue(*steps):
    live = [[lo, i, lo, hi, step] for i, (lo, hi, step) in enumerate(steps)]
    while live:
        cur = min(live, key=lambda g: g[:2])
        f = next(cur[4], None)
        if f is None:
            live.remove(cur)
        else:
            cur[0] = cur[2] + f * (cur[3] - cur[2])


def _run(*steps):
    _issue(*[(0, 1, step) for step in steps])


def _dot(a, b):
    return jnp.dot(a, b, preferred_element_type=F32)


def _add(values):
    return functools.reduce(lambda a, b: a + b, values)


def _tile(j):
    return slice(j * T, (j + 1) * T)


def _standardize(x):
    d = x.shape[-1]
    xc = x - jnp.sum(x, axis=-1, keepdims=True) * (1.0 / d)
    var = jnp.sum(xc * xc, axis=-1, keepdims=True) * (1.0 / d)
    return xc * lax.rsqrt(var + 1e-5)


def _phi(t):
    return jnp.where(t > 0, t + 1.0, jnp.exp(t)) + 1e-6


def _kernel(x_hbm, wqkv_hbm, wo_hbm, wg_hbm, wu_hbm, wd_hbm, c_hbm, wmod_hbm, out_hbm,
            x_v, wqkv_v, wo_v, wg_v, wu_v, wd_v, c_v, wmod_v, out_v,
            wq_t, m_v, z_t, zs_t, mod_v, n_v, pk_v, q_v, w_ops, carry_v, in_sems, out_sems):
    S, D = x_v.shape
    F = wd_v.shape[0]
    r1, r2, n1, n2 = R1 // 2, R2 // 2, S // R1, S // R2
    dh, per = D // HEADS, T // HEADS
    nf = F // T
    tail = F - nf * T
    groups = [[('g', i) for i in range(0, 5)], [('u', i) for i in range(0, 5)],
              [('g', i) for i in range(5, 10)], [('u', i) for i in range(5, 10)],
              [('g', 10), ('u', 10), ('g', 11), ('u', 11), ('g', 12)]]
    last, last_plain = [('u', 12), ('m', nf)], 4
    last_products = [(ks, p) for ks in ((0, 2), (1, 3)) for p in range(P) if _C[p].reshape(NT, NT)[np.ix_(ks, ks)].any()]
    NG = len(groups)
    left_sums, right_sums = _Sums(_U, False), _Sums(_C, True)
    out_sums = {True: _Sums(_X.T), False: _Sums(_X.T, False)}
    cut = mod_v.shape[1]
    st = {}

    cols = lambda a, b: (slice(None), pl.ds(a, b - a))
    rows = lambda a, n: (pl.ds(a, n), slice(None))
    whole = (slice(None), slice(None))
    loads = {'c': (c_hbm, c_v, whole), 'wo': (wo_hbm, wo_v, whole), 'wg': (wg_hbm, wg_v, whole),
             'wu': (wu_hbm, wu_v, whole), 'wd': (wd_hbm, wd_v, whole), 'mod_0': (wmod_hbm, wmod_v, cols(0, cut)),
             'mod_1': (wmod_hbm, wmod_v, cols(cut, 2 * D)), 'mod_b': (wmod_hbm, wmod_v, cols(2 * D, 6 * D))}
    for i, name in enumerate(('wq', 'wk', 'wv')):
        loads[name] = (wqkv_hbm, wqkv_v, cols(i * D, (i + 1) * D))
    for i in range(n1):
        loads['x%d' % i] = (x_hbm, x_v, rows(i * R1, R1))

    def copy_in(name):
        hbm, vmem, part = loads[name]
        return pltpu.make_async_copy(hbm.at[part], vmem.at[part], in_sems.at[list(loads).index(name)])

    def wait(names):
        for name in names.split():
            copy_in(name).wait()

    def operands(sums, tiles):
        return [None if v is None else v.astype(BF16) for v in sums.of(tiles)]

    def weights(tile):
        return operands(right_sums, [tile(k, n) for k in range(NT) for n in range(NT)])

    def put_transposed(slot, i, v):
        w_ops[slot, i] = pltpu.bitcast(v.astype(BF16).T, U32)

    def put_weights(slot, tile_t):
        for p, v in enumerate(right_sums.of([tile_t(k, n).astype(F32) for k in range(NT) for n in range(NT)])):
            put_transposed(slot, p, v)
            yield (p + 1) / P

    def stored(slot, i):
        return pltpu.bitcast(w_ops[slot, i], BF16)

    def matmul(kind, product, emit):
        push = out_sums[kind[0] in 'kqgua'].stream()
        for done, p in enumerate(_ORDER.get(kind) or _ORDER[kind[0]]):
            for i, v in push(p, product(p)):
                emit(i // 2, i % 2, v)
            yield (done + 1) / P

    def silu_c():
        c = c_v[...].astype(F32)
        return jnp.broadcast_to(c / (1.0 + jnp.exp(-c)), (16, D)).astype(BF16)

    def prepare_q():
        for k in range(NT):
            for n in range(NT):
                wq_t[k, _tile(n), :] = wqkv_v[_tile(k), _tile(n)].astype(F32).T
        st['wq'] = weights(lambda k, n: jnp.concatenate(
            [wq_t[k, pl.ds(d, HEADS, stride=dh), :] for d in range(n * per, (n + 1) * per)], axis=0).T)

    def norm1(t):
        x = n_v[...] if t == 0 else _standardize(x_v[t * R1:(t + 1) * R1, :].astype(F32))
        h = x * st['ca'] + st['sa']
        st['h', t] = operands(left_sums, [h[m * r1:(m + 1) * r1, _tile(k)] for k in range(NT) for m in range(2)])

    def project(t, which):
        def emit(n, m, v):
            at = (pl.ds(t * R1 + m * r1, r1), _tile(n))
            if which == 'q':
                q_v[at] = v
                return
            v = _phi(v)
            if t == 0:
                st['k', n, m] = v
            else:
                pk_v[at] = v * st['scale'][:, _tile(n)]
            s = jnp.sum(v.reshape(-1, 8, T), axis=0)
            st['z', n] = st['z', n] + s if ('z', n) in st else s
        return matmul(which + str(t), lambda p: _dot(st['h', t][p], st['w' + which][p]), emit)

    def column_sums():
        return jnp.concatenate([jnp.sum(st['z', n], axis=0, keepdims=True) for n in range(NT)], axis=1)

    def scale_columns():
        st['scale'] = 1.0 / column_sums()
        for n in range(NT):
            for m in range(2):
                pk_v[m * r1:(m + 1) * r1, _tile(n)] = st['k', n, m] * st['scale'][:, _tile(n)]

    def finish_sums():
        z = column_sums()
        zs_t[...] = jnp.broadcast_to(1.0 / (z * st['scale']), (T, D)).T
        z_t[0:D, :] = jnp.broadcast_to(z, (T, D)).T
        st['z'] = jnp.concatenate([z_t[pl.ds(d, HEADS, stride=dh), :] for d in range(dh)], axis=0).T[0:1]

    def gram():
        push = _Sums(_C.T, True).stream()
        for done, p in enumerate(_ORDER['G']):
            def term(t):
                pk = _signed_sum([(pk_v[pl.ds(t * R1 + m * r1, r1), _tile(n)], int(_X[p, 2 * n + m]))
                                  for n in range(NT) for m in range(2) if _X[p, 2 * n + m]])
                return lax.dot_general(pk.astype(BF16), st['h', t][p], (((0,), (0,)), ((), ())),
                                       preferred_element_type=F32)
            for i, v in push(p, _add([term(t) for t in range(n1)])):
                st['g', i % NT, i // NT] = v
            yield (done + 1) / P

    def fold():
        g = jnp.concatenate([jnp.concatenate([st['g', i, j] for j in range(NT)], axis=1) for i in range(NT)], axis=0)
        done = 0
        for j in range(NT):
            lo = (j * T // dh * dh) // 16 * 16
            hi = pl.cdiv(pl.cdiv((j + 1) * T, dh) * dh, 16) * 16
            kv = _dot(g[lo:hi].astype(BF16), wqkv_v[:, _tile(2 * NT + j)])
            head = lambda axis, first: jnp.floor(
                ((lax.broadcasted_iota(jnp.int32, kv.shape, axis) + first).astype(F32) + 0.5) * (1.0 / dh))
            kv = jnp.where(head(0, lo) == head(1, j * T), kv, 0.0) * zs_t[lo:hi, :]
            m = _dot(kv.astype(BF16), wo_v[_tile(j), :])
            for n in range(NT):
                if lo < done:
                    m_v[n, lo:done, :] += m[:done - lo, _tile(n)]
                m_v[n, done:hi, :] = m[done - lo:, _tile(n)]
            done = hi
            yield (j + 1) / NT

    def modulate():
        sc, tiles = silu_c(), []
        for j in range(4 * NT):
            tiles.append(_dot(sc, wmod_v[:, _tile(2 * NT + j)])[0:1])
            yield (j + 1) / (4 * NT)
        st['ga'], sb, cb, gb = (jnp.concatenate(tiles[i * NT:(i + 1) * NT], axis=1) for i in range(4))
        st['sb'], st['cb'], st['gb'] = 0.5 * sb, 0.5 + 0.5 * cb, 2.0 * gb

    def hidden_tile_t(kind, i, k):
        if kind == 'm':
            return jnp.concatenate([wg_v[nf * T:F, _tile(k)], wu_v[nf * T:F, _tile(k)]], axis=0)
        return (wg_v if kind == 'g' else wu_v)[_tile(i), _tile(k)]

    def prepare_hidden(g):
        if g < NG:
            yield from put_weights(g, lambda k, n: hidden_tile_t(*groups[g][n], k))
            return
        for i, (ks, p) in enumerate(last_products):
            put_transposed(NG, i, _signed_sum([(hidden_tile_t(*last[n], k).astype(F32), int(_C[p, k * NT + ks[n]]))
                                               for k in ks for n in range(2) if _C[p, k * NT + ks[n]]]))
        for n in range(2):
            put_transposed(NG, len(last_products) + n, hidden_tile_t(*last[n], last_plain))

    def down_tile(g, k, n):
        lo = (g * NT + k) * T
        w = wd_v[lo:min(lo + T, F), _tile(n)]
        return w if lo + T <= F else jnp.concatenate([w, jnp.zeros((lo + T - F, T), BF16)], axis=0)

    def prepare_down(g):
        return put_weights(NG + 1 + g, lambda k, n: down_tile(g, k, n).T if (g * NT + k) * T < F else jnp.zeros((T, T), BF16))

    def down_used(g, p):
        ks = [k for k in range(NT) if (g * NT + k) * T < F]
        return _U[p].reshape(NT, 2)[ks].any() and _C[p].reshape(NT, NT)[ks].any()

    def attend(first):
        at = lambda m: pl.ds(first + m * r2, r2)
        tiles = {}
        for m in range(2):
            w = [_phi(q_v[at(m), _tile(n)]) * st['z'][:, _tile(n)] for n in range(NT)]
            s = _add(w)
            s = s + pltpu.roll(s, 64, 1)
            s = s + pltpu.roll(s, 32, 1)
            inv = 1.0 / (s + 1e-6)
            for n in range(NT):
                tiles[n, m] = w[n] * inv
        ops = operands(left_sums, [tiles[n, m] for n in range(NT) for m in range(2)])
        x1 = {}

        def emit(n, m, v):
            x1[n, m] = x_v[at(m), _tile(n)].astype(F32) + v
        yield from matmul('a', lambda p: _dot(ops[p], st['wm'][p]), emit)
        for m in range(2):
            x = jnp.concatenate([x1[n, m] for n in range(NT)], axis=1)
            carry_v[0, m] = _standardize(x) * st['cb'] + st['sb']
            carry_v[1, m] = x

    def feed_forward(first, more):
        x1 = {(n, m): carry_v[1, m, :, _tile(n)] for m in range(2) for n in range(NT)}
        h2 = [carry_v[0, m] for m in range(2)]
        tiles = [h2[m][:, _tile(k)] for k in range(NT) for m in range(2)]
        ops = operands(left_sums, tiles)
        plain = [v.astype(BF16) for v in tiles[2 * last_plain:2 * last_plain + 2]]
        held, act = {}, []

        def emit(kind, i, m, v):
            if kind == 'm':
                a = v * pltpu.roll(v, tail, 1) * (1.0 + jnp.tanh(v))
                held['a', i, m] = jnp.where(lax.broadcasted_iota(jnp.int32, v.shape, 1) < tail, a, 0.0)
                return
            held[kind, i, m] = v * (1.0 + jnp.tanh(v)) if kind == 'g' else v
            if ('g', i, m) in held and ('u', i, m) in held:
                held['a', i, m] = held['g', i, m] * held['u', i, m]

        def group(g):
            _run(matmul('gu'[g % 2], lambda p: _dot(ops[p], stored(g, p)), lambda n, m, v: emit(*groups[g][n], m, v)))

        def activations(g):
            act.append(operands(left_sums, [held.get(('a', g * NT + k, m)) for k in range(NT) for m in range(2)]))

        for g in range(2):
            group(2 * g)
            group(2 * g + 1)
            activations(g)
        terms = {(n, m): [] for n in range(2) for m in range(2)}
        for i, (ks, p) in enumerate(last_products):
            v = _dot(ops[p], stored(NG, i))
            for n, m in terms:
                if _X[p, 2 * ks[n] + m]:
                    terms[n, m].append((v, int(_X[p, 2 * ks[n] + m])))
        for n, m in terms:
            v = _dot(plain[m], stored(NG, len(last_products) + n))
            emit(*last[n], m, _signed_sum(terms[n, m] + [(v, 1)]))
        group(4)
        activations(2)
        if more:
            _run(attend(first + R2))

        def put(n, m, v):
            out_v[pl.ds(first + m * r2, r2), _tile(n)] = (x1[n, m] + st['gb'][:, _tile(n)] * v).astype(BF16)
        _run(matmul('d', lambda p: _add([_dot(act[g][p], stored(NG + 1 + g, p)) for g in range(3) if down_used(g, p)]), put))

    def copy_out(t, first):
        return pltpu.make_async_copy(out_v.at[rows(first, R2)], out_hbm.at[rows(first, R2)], out_sems.at[t])

    xs = lambda a, b: ' '.join('x%d' % i for i in range(a, b))
    for name in ('c wq x0 mod_0 mod_1 x1 wk ' + xs(2, n1) + ' wg wu wd mod_b wv wo').split():
        copy_in(name).start()
    for ref in (wq_t, m_v):
        ref[:, D:, :] = jnp.zeros((NT, ref.shape[1] - D, T), F32)
    z_t[D:, :] = jnp.zeros((z_t.shape[0] - D, T), F32)
    wait('c wq')
    prepare_q()
    wait('x0')
    n_v[...] = _standardize(x_v[0:R1, :].astype(F32))
    sc = silu_c()
    wait('mod_0')
    mod_v[...] = _dot(sc, wmod_v[:, 0:cut])[0:1]
    wait('mod_1')
    mod = jnp.concatenate([mod_v[...], _dot(sc, wmod_v[:, cut:2 * D])[0:1]], axis=1)
    st['sa'], st['ca'] = mod[:, 0:D], 1.0 + mod[:, D:2 * D]

    at = lambda f, fn, *args: (f, f, _once(fn, *args))
    norm1(0)
    _issue((0, 1, project(0, 'q')), at(0.5, wait, 'x1'))
    norm1(1)
    _issue((0, 1, project(1, 'q')), at(0.8, wait, 'wk x2'))
    st['wk'] = weights(lambda k, n: wqkv_v[_tile(k), _tile(NT + n)].astype(F32))
    _run(project(0, 'k'))
    scale_columns()
    _run(project(1, 'k'))
    late = list(range(n1 - 3, n1))
    for t in range(2, n1):
        norm1(t)
        _issue((0, 1, project(t, 'k')), *([at(0.9, wait, xs(3, n1))] if t == 2 else []))
        if t not in late:
            _run(project(t, 'q'))
    _issue((0, 1, project(late.pop(0), 'q')), at(0.3, wait, 'wg wu'))
    hidden = lambda gs: [(1 if g < NG else 0.3, prepare_hidden(g)) for g in gs]
    down = lambda gs: [(1, prepare_down(g)) for g in gs]
    _issue((0, 1, gram()), (0, 1, _chain(*hidden((0, 1, 2, 3)))),
           at(1.01, wait, 'wd mod_b wv wo'), at(0.9, finish_sums))
    spare_q = lambda: project(late.pop(0), 'q')
    _issue((0, 1, _chain((2, fold()), (1, modulate()))),
           (0, 1, _chain(*hidden((4, 5)), *down(range(3)))),
           (0, 1, spare_q()))
    st['wm'] = weights(lambda k, n: jnp.concatenate(
        [m_v[n, pl.ds(d, HEADS, stride=dh), :] for d in range(k * per, (k + 1) * per)], axis=0) * st['ga'][:, _tile(n)])
    _run(attend(0), spare_q())

    def body(t, carry):
        first = pl.multiple_of(t * R2, R2)
        feed_forward(first, True)
        copy_out(t, first).start()
        return carry

    lax.fori_loop(0, n2 - 1, body, 0)
    feed_forward(S - R2, False)
    copy_out(n2 - 1, S - R2).start()
    for t in range(n2):
        copy_out(t, t * R2).wait()


@jax.jit
def pallas_adaLN_cond__linear_attn_block__swiglu_ffn__prompt_kernel(
    A_x: jax.Array,
    A_wqkv: jax.Array,
    A_wo: jax.Array,
    B_x: jax.Array,
    B_w_gate: jax.Array,
    B_w_up: jax.Array,
    B_w_down: jax.Array,
    c: jax.Array,
    w_mod: jax.Array,
):
    del B_x
    B, S, D = A_x.shape
    F = B_w_gate.shape[1]
    assert B == 1 and D == NT * T and F == 27 * T // 2 and S % R1 == 0 and S >= 6 * R1
    pad = 2 * D // HEADS
    vm = pltpu.VMEM
    hbm = pl.BlockSpec(memory_space=pltpu.HBM)
    out = pl.pallas_call(
        _kernel,
        out_shape=jax.ShapeDtypeStruct((S, D), A_x.dtype),
        in_specs=[hbm] * 8,
        out_specs=hbm,
        scratch_shapes=[
            vm((S, D), BF16), vm((D, 3 * D), BF16), vm((D, D), BF16), vm((F, D), BF16), vm((F, D), BF16),
            vm((F, D), BF16), vm((1, D), BF16), vm((D, 6 * D), BF16), vm((S, D), BF16),
            vm((NT, D + pad, T), F32), vm((NT, D + pad, T), F32), vm((D + pad, T), F32), vm((D, T), F32),
            vm((1, 8 * T), F32), vm((R1, D), F32), vm((S, D), F32), vm((S, D), F32),
            vm((9, P, T // 2, T), U32), vm((2, 2, R2 // 2, D), F32),
            pltpu.SemaphoreType.DMA((11 + S // R1,)), pltpu.SemaphoreType.DMA((S // R2,)),
        ],
        compiler_params=pltpu.CompilerParams(vmem_limit_bytes=100 * 2**20),
        name='adaln_block',
    )(A_x.reshape(S, D), A_wqkv, A_wo, B_w_gate.T, B_w_up.T, B_w_down, c, w_mod)
    return out.reshape(B, S, D)
```
